```python
import os as _os
_os.environ.setdefault("JAX_PLATFORMS", "cpu")
import jax
import jax.numpy as jnp

def _softmax(x, axis=-1):
    return jax.nn.softmax(x, axis=axis)
def _gelu(x):
    return jax.nn.gelu(x, approximate=True)
def _silu(x):
    return jax.nn.silu(x)
def _sigmoid(x):
    return jax.nn.sigmoid(x)
def _layernorm(x, axis=-1, eps=1e-5):
    m = jnp.mean(x, axis=axis, keepdims=True)
    v = jnp.var(x, axis=axis, keepdims=True)
    return (x - m) / jnp.sqrt(v + eps)
def _scatter_add(tgt, idx, src, axis=0):
    return tgt.at[idx].add(src)
def _segment_sum(src, seg, n):
    return jax.ops.segment_sum(src, seg, n)
class _Rng:
    def __init__(self, key):
        self._k = key
    def _next(self):
        self._k, sub = jax.random.split(self._k)
        return sub
    def normal(self, shape):
        return jax.random.normal(self._next(), shape, dtype=jnp.bfloat16)
    def randint(self, lo, hi, shape):
        return jax.random.randint(self._next(), shape, lo, hi, dtype=jnp.int32)
    def uniform(self, shape, lo=0.0, hi=1.0):
        return jax.random.uniform(self._next(), shape, jnp.bfloat16, lo, hi)
    def permutation(self, n):
        return jax.random.permutation(self._next(), n)


kernel_name = 'sequential_preLN__ssm_conv_h3__mixer_s_mlp__prompt'

def setup_inputs():
    _rng = _Rng(jax.random.key(int.from_bytes(__import__("os").urandom(4), "little")))
    _w = (lambda a: (lambda t: t.astype(jnp.bfloat16) if jnp.issubdtype(t.dtype, jnp.floating) else t)(jnp.asarray(a)))
    def _A_setup():
        B, S, D = 1, 2048, 640
        ks = 4
        return {
            "q": _w((lambda *s: _rng.normal(s) * 0.05)(B, S, D)),
            "k": _w((lambda *s: _rng.normal(s) * 0.05)(B, S, D)),
            "v": _w((lambda *s: _rng.normal(s) * 0.05)(B, S, D)),
            "shift_k": _w((lambda *s: _rng.normal(s) * 0.05)(D, ks) * 0.5),
            "ssm_k": _w((lambda *s: _rng.normal(s) * 0.05)(D, S) * (1.0 / S ** 0.5)),
            "ssm_D": _w((lambda *s: _rng.normal(s) * 0.05)(D)),
        }
    _A_in = _A_setup()

    def _B_setup():
        B, S, D, F = 1, 2048, 640, 1728
        return {
            "x":  _w((lambda *s: _rng.normal(s) * 0.05)(B, S, D)),
            "w1": _w((lambda *s: _rng.normal(s) * 0.8)(D, D) * (D ** -0.5)),
            "w2": _w((lambda *s: _rng.normal(s) * 0.8)(D, D) * (D ** -0.5)),
            "w3": _w((lambda *s: _rng.normal(s) * 0.8)(D, F) * (D ** -0.5)),
            "w4": _w((lambda *s: _rng.normal(s) * 0.8)(F, D) * (F ** -0.5)),
        }
    _B_in = _B_setup()

    return {
        "A_q": _A_in["q"],
        "A_k": _A_in["k"],
        "A_v": _A_in["v"],
        "A_shift_k": _A_in["shift_k"],
        "A_ssm_k": _A_in["ssm_k"],
        "A_ssm_D": _A_in["ssm_D"],
        "B_x": _B_in["x"],
        "B_w1": _B_in["w1"],
        "B_w2": _B_in["w2"],
        "B_w3": _B_in["w3"],
        "B_w4": _B_in["w4"],
    }

def reference(A_q, A_k, A_v, A_shift_k, A_ssm_k, A_ssm_D, B_x, B_w1, B_w2, B_w3, B_w4):
    def _A_ref(q, k, v, shift_k, ssm_k, ssm_D):
        B, S, D = q.shape
        ks = shift_k.shape[-1]
        k_pad = jnp.pad(k, ((0, 0), (ks - 1, 0), (0, 0)))
        k_shift = jnp.zeros_like(k)
        for t in range(ks):
            k_shift = k_shift + k_pad[:, t:t + S, :] * shift_k[:, ks - 1 - t][None, None, :]
        kv = k_shift * v
        L = 2 * S
        kv_pad = jnp.pad(kv, ((0, 0), (0, S), (0, 0)))
        kf_pad = jnp.pad(ssm_k, ((0, 0), (0, S)))
        kv_f = (lambda x, axes=(-2,-1): jnp.fft.rfft2(x.astype(jnp.float32), axes=axes))(kv_pad[:, None, :, :], axes=(1, 2))
        kf_f = (lambda x, axes=(-2,-1): jnp.fft.rfft2(x.astype(jnp.float32), axes=axes))(kf_pad[:, None, :], axes=(1, 2))
        kf_f = (lambda x, *d: x.transpose(*d))(kf_f, 1, 2, 0)
        y_f = kv_f * kf_f[None, :, :, :]
        y = (lambda x, s, axes=(-2,-1): jnp.fft.irfft2(x, s=s, axes=axes).astype(jnp.bfloat16))(y_f, (1, L), axes=(1, 2))[:, 0, :S, :]
        y = y + kv * ssm_D[None, None, :]
        return q * y

    def _B_ref(x, w1, w2, w3, w4):
        B, S, D = x.shape
        h = _gelu(_layernorm(x, axis=-1) @ w1)
        c = D // 4
        g0 = jnp.pad(h[:, :, 0*c:1*c], ((0, 0), (1, 0), (0, 0)))[:, :S, :]
        g1 = jnp.pad(h[:, :, 1*c:2*c], ((0, 0), (0, 1), (0, 0)))[:, 1:, :]
        g2 = jnp.pad(h[:, :, 2*c:3*c], ((0, 0), (2, 0), (0, 0)))[:, :S, :]
        g3 = jnp.pad(h[:, :, 3*c:   ], ((0, 0), (0, 2), (0, 0)))[:, 2:, :]
        hs = jnp.concatenate([g0, g1, g2, g3], axis=-1) @ w2
        x1 = x + hs
        h2 = _gelu(_layernorm(x1, axis=-1) @ w3) @ w4
        return x1 + h2

    x = A_q
    h = x + _A_ref(_layernorm(x, axis=-1), A_k, A_v, A_shift_k, A_ssm_k, A_ssm_D)
    h2 = h + _B_ref(_layernorm(h, axis=-1), B_w1, B_w2, B_w3, B_w4)
    return h2
```

```python
import numpy as np
import jax
import jax.numpy as jnp
import jax.experimental.pallas as pl
import jax.experimental.pallas.tpu as pltpu

_EPS = 1e-5
_HALO = 8


def _dft_mats(C):
    n = np.arange(C)[None, :]
    f = np.arange(C)[:, None]
    ang = np.pi * n * (2 * f + 1) / (2 * C)
    fx = np.concatenate([np.cos(ang), -np.sin(ang)], 0)
    t = (np.arange(C) + C)[:, None]
    f2 = np.arange(C)[None, :]
    th = np.pi * t * (2 * f2 + 1) / (2 * C)
    finv = np.concatenate([np.cos(th), -np.sin(th)], 1) / C
    return fx.astype(np.float32), finv.astype(np.float32)


def _ln(x):
    m = jnp.mean(x, axis=-1, keepdims=True)
    xc = x - m
    v = jnp.mean(xc * xc, axis=-1, keepdims=True)
    return xc * jax.lax.rsqrt(v + _EPS)


def _gelu(x):
    return jax.nn.gelu(x, approximate=True)


def _make_kernel(S, D, FF, C, TM, RC):
    NT = S // TM
    CPB = TM // C
    c4 = D // 4

    def kernel(q_ref, k_ref, v_ref, kt_ref, sh_ref, dv_ref,
               w1_ref, w2_ref, w3_ref, w4_ref, fx_ref, finv_ref,
               out_ref,
               xf_scr, kf_scr, tprev_scr, kcarry_scr, h_scr, hh_scr):
        i = pl.program_id(0)

        @pl.when(i == 0)
        def _init():
            tprev_scr[...] = jnp.zeros(tprev_scr.shape, jnp.float32)
            kcarry_scr[...] = jnp.zeros(kcarry_scr.shape, jnp.float32)
            hh_scr[pl.ds(0, _HALO), :] = jnp.zeros((_HALO, D), jnp.float32)
            hh_scr[pl.ds(_HALO + S, _HALO), :] = jnp.zeros((_HALO, D), jnp.float32)

        @pl.when(i < NT)
        def _phase_a():
            x = q_ref[...].astype(jnp.float32)
            k = k_ref[...].astype(jnp.float32)
            v = v_ref[...].astype(jnp.float32)
            kk = jnp.concatenate([kcarry_scr[...], k], axis=0)
            kcarry_scr[...] = k[TM - 8:, :]
            sh = sh_ref[...]
            ks = (kk[5:5 + TM] * sh[3:4] + kk[6:6 + TM] * sh[2:3]
                  + kk[7:7 + TM] * sh[1:2] + kk[8:8 + TM] * sh[0:1])
            kv = (ks * v).astype(jnp.bfloat16)
            fx = fx_ref[...]
            finv = finv_ref[...]
            sgn = (1.0 - 2.0 * (jax.lax.broadcasted_iota(jnp.int32, (C, D), 0) % 2)
                   ).astype(jnp.float32)
            kt = kt_ref[...]
            ys = []
            for cb in range(CPB):
                jb = i * CPB + cb
                xf_scr[jb] = jnp.dot(fx, kv[cb * C:(cb + 1) * C],
                                     preferred_element_type=jnp.float32)
                tm = jnp.dot(fx, kt[cb * C:(cb + 1) * C],
                             preferred_element_type=jnp.float32)
                tp = tprev_scr[...]
                kf_scr[jb, pl.ds(0, C), :] = tp[:C] + sgn * tm[C:]
                kf_scr[jb, pl.ds(C, C), :] = tp[C:] - sgn * tm[:C]
                tprev_scr[...] = tm
                yr_parts = []
                yi_parts = []
                for rc in range(C // RC):
                    r0 = rc * RC

                    def body(j, carry, r0=r0, jb=jb):
                        ar, ai = carry
                        m = jb - j
                        kr = kf_scr[m, pl.ds(r0, RC), :]
                        ki = kf_scr[m, pl.ds(C + r0, RC), :]
                        xr = xf_scr[j, pl.ds(r0, RC), :]
                        xi = xf_scr[j, pl.ds(C + r0, RC), :]
                        ar = ar + (kr * xr - ki * xi)
                        ai = ai + (kr * xi + ki * xr)
                        return ar, ai

                    z = jnp.zeros((RC, D), jnp.float32)
                    ar, ai = jax.lax.fori_loop(0, jb + 1, body, (z, z))
                    yr_parts.append(ar)
                    yi_parts.append(ai)
                yf = jnp.concatenate(yr_parts + yi_parts, axis=0).astype(jnp.bfloat16)
                ys.append(jnp.dot(finv, yf, preferred_element_type=jnp.float32))
            y = jnp.concatenate(ys, axis=0) if CPB > 1 else ys[0]
            y = y.astype(jnp.bfloat16).astype(jnp.float32)
            y = y + kv.astype(jnp.float32) * dv_ref[...]
            h = x + _ln(x) * y
            row = pl.multiple_of(i * TM, TM)
            h_scr[pl.ds(row, TM), :] = h
            xb = _ln(h)
            u = _ln(xb).astype(jnp.bfloat16)
            hh = _gelu(jnp.dot(u, w1_ref[...], preferred_element_type=jnp.float32))
            hh_scr[pl.ds(pl.multiple_of(_HALO + i * TM, 8), TM), :] = hh

        @pl.when(i >= 1)
        def _phase_b():
            b = i - 1
            row = pl.multiple_of(b * TM, TM)
            win = hh_scr[pl.ds(row, TM + 2 * _HALO), :]
            col = jax.lax.broadcasted_iota(jnp.int32, (TM, D), 1)
            hp1 = win[_HALO - 1:_HALO - 1 + TM]
            hm1 = win[_HALO + 1:_HALO + 1 + TM]
            hp2 = win[_HALO - 2:_HALO - 2 + TM]
            hm2 = win[_HALO + 2:_HALO + 2 + TM]
            g = jnp.where(col < c4, hp1,
                          jnp.where(col < 2 * c4, hm1,
                                    jnp.where(col < 3 * c4, hp2, hm2)))
            hs = jnp.dot(g.astype(jnp.bfloat16), w2_ref[...],
                         preferred_element_type=jnp.float32)
            h = h_scr[pl.ds(row, TM), :]
            xb = _ln(h)
            x1 = xb + hs
            u = _ln(x1).astype(jnp.bfloat16)
            a = _gelu(jnp.dot(u, w3_ref[...], preferred_element_type=jnp.float32))
            h2 = jnp.dot(a.astype(jnp.bfloat16), w4_ref[...],
                         preferred_element_type=jnp.float32)
            out_ref[...] = (h + x1 + h2).astype(out_ref.dtype)

    return kernel


@jax.jit
def pallas_sequential_preLN__ssm_conv_h3__mixer_s_mlp__prompt_kernel(
    A_q: jax.Array,
    A_k: jax.Array,
    A_v: jax.Array,
    A_shift_k: jax.Array,
    A_ssm_k: jax.Array,
    A_ssm_D: jax.Array,
    B_x: jax.Array,
    B_w1: jax.Array,
    B_w2: jax.Array,
    B_w3: jax.Array,
    B_w4: jax.Array,
):
    B, S, D = A_q.shape
    assert B == 1
    FF = B_w3.shape[1]
    ks = A_shift_k.shape[1]
    assert ks == 4
    C = 128
    TM = 256
    RC = 32
    NT = S // TM
    NB = S // C

    q2 = A_q.reshape(S, D)
    k2 = A_k.reshape(S, D)
    v2 = A_v.reshape(S, D)
    kt = A_ssm_k.T
    sh = jnp.pad(A_shift_k.T.astype(jnp.float32), ((0, 8 - ks), (0, 0)))
    dv = A_ssm_D.reshape(1, D).astype(jnp.float32)
    fx_np, finv_np = _dft_mats(C)
    fx = jnp.asarray(fx_np, dtype=jnp.bfloat16)
    finv = jnp.asarray(finv_np, dtype=jnp.bfloat16)

    row_in = lambda i: (jnp.minimum(i, NT - 1), 0)
    row_out = lambda i: (jnp.maximum(i - 1, 0), 0)
    const = lambda i: (0, 0)

    kernel = _make_kernel(S, D, FF, C, TM, RC)
    out = pl.pallas_call(
        kernel,
        grid_spec=pltpu.PrefetchScalarGridSpec(
            num_scalar_prefetch=0,
            grid=(NT + 1,),
            in_specs=[
                pl.BlockSpec((TM, D), row_in),
                pl.BlockSpec((TM, D), row_in),
                pl.BlockSpec((TM, D), row_in),
                pl.BlockSpec((TM, D), row_in),
                pl.BlockSpec((8, D), const),
                pl.BlockSpec((1, D), const),
                pl.BlockSpec((D, D), const),
                pl.BlockSpec((D, D), const),
                pl.BlockSpec((D, FF), const),
                pl.BlockSpec((FF, D), const),
                pl.BlockSpec((2 * C, C), const),
                pl.BlockSpec((C, 2 * C), const),
            ],
            out_specs=pl.BlockSpec((TM, D), row_out),
            scratch_shapes=[
                pltpu.VMEM((NB, 2 * C, D), jnp.float32),
                pltpu.VMEM((NB, 2 * C, D), jnp.float32),
                pltpu.VMEM((2 * C, D), jnp.float32),
                pltpu.VMEM((8, D), jnp.float32),
                pltpu.VMEM((S, D), jnp.float32),
                pltpu.VMEM((S + 2 * _HALO, D), jnp.float32),
            ],
        ),
        out_shape=jax.ShapeDtypeStruct((S, D), A_q.dtype),
        compiler_params=pltpu.CompilerParams(
            dimension_semantics=("arbitrary",),
            vmem_limit_bytes=100 * 1024 * 1024,
        ),
    )(q2, k2, v2, kt, sh, dv, B_w1, B_w2, B_w3, B_w4, fx, finv)
    return out.reshape(B, S, D)
```

```python
import numpy as np
import jax
import jax.numpy as jnp
import jax.experimental.pallas as pl
import jax.experimental.pallas.tpu as pltpu

_EPS = 1e-5
_HALO = 8


def _dft_mats(C):
    n = np.arange(C)[None, :]
    f = np.arange(C)[:, None]
    ang = np.pi * n * (2 * f + 1) / (2 * C)
    fx = np.concatenate([np.cos(ang), -np.sin(ang)], 0)
    t = (np.arange(C) + C)[:, None]
    f2 = np.arange(C)[None, :]
    th = np.pi * t * (2 * f2 + 1) / (2 * C)
    finv = np.concatenate([np.cos(th), -np.sin(th)], 1) / C
    return fx.astype(np.float32), finv.astype(np.float32)


def _ln(x):
    m = jnp.mean(x, axis=-1, keepdims=True)
    xc = x - m
    v = jnp.mean(xc * xc, axis=-1, keepdims=True)
    return xc * jax.lax.rsqrt(v + _EPS)


def _gelu(x):
    return jax.nn.gelu(x, approximate=True)


def _make_kernel(S, D, FF, C, TM, RC):
    NT = S // TM
    assert TM == 2 * C
    c4 = D // 4

    def kernel(q_ref, k_ref, v_ref, kt_ref, sh_ref, dv_ref,
               w1_ref, w2_ref, w3_ref, w4_ref, fx_ref, finv_ref,
               out_ref,
               xf_scr, kf_scr, tprev_scr, kcarry_scr, h_scr, hh_scr, y_scr,
               w1_scr, w2_scr, w3_scr, w4_scr, wsem, w3t_scr, xb_scr):
        i = pl.program_id(0)

        def wcopy(n):
            src, dst = ((w1_ref, w1_scr), (w2_ref, w2_scr), (w3_ref, w3t_scr), (w4_ref, w4_scr))[n]
            return pltpu.make_async_copy(src, dst, wsem.at[n])
        ja = 2 * i

        @pl.when(i == 0)
        def _init():
            for n in range(4):
                wcopy(n).start()
            tprev_scr[...] = jnp.zeros(tprev_scr.shape, jnp.float32)
            kcarry_scr[...] = jnp.zeros(kcarry_scr.shape, jnp.float32)
            hh_scr[pl.ds(0, _HALO), :] = jnp.zeros((_HALO, D), jnp.float32)
            hh_scr[pl.ds(_HALO + S, _HALO), :] = jnp.zeros((_HALO, D), jnp.float32)

        @pl.when(i < NT)
        def _phase_a():
            k = k_ref[...].astype(jnp.float32)
            v = v_ref[...].astype(jnp.float32)
            kk = jnp.concatenate([kcarry_scr[...], k], axis=0)
            kcarry_scr[...] = k[TM - 8:, :]
            sh = sh_ref[...]
            ks = (kk[5:5 + TM] * sh[3:4] + kk[6:6 + TM] * sh[2:3]
                  + kk[7:7 + TM] * sh[1:2] + kk[8:8 + TM] * sh[0:1])
            kv = (ks * v).astype(jnp.bfloat16)
            fx = fx_ref[...]
            sgn = (1.0 - 2.0 * (jax.lax.broadcasted_iota(jnp.int32, (C, D), 0) % 2)
                   ).astype(jnp.float32)
            kt = kt_ref[...]
            for cb in range(2):
                jb = ja + cb
                xf_scr[jb] = jnp.dot(fx, kv[cb * C:(cb + 1) * C],
                                     preferred_element_type=jnp.float32)
                tm = jax.lax.dot_general(fx, kt[:, cb * C:(cb + 1) * C],
                                         (((1,), (1,)), ((), ())),
                                         preferred_element_type=jnp.float32)
                tp = tprev_scr[...]
                kf_scr[jb, pl.ds(0, C), :] = tp[:C] + sgn * tm[C:]
                kf_scr[jb, pl.ds(C, C), :] = tp[C:] - sgn * tm[:C]
                tprev_scr[...] = tm
            xr = xf_scr[ja + 1, pl.ds(0, C), :]
            xi = xf_scr[ja + 1, pl.ds(C, C), :]
            kr = kf_scr[0, pl.ds(0, C), :]
            ki = kf_scr[0, pl.ds(C, C), :]
            y_scr[0] = jnp.zeros((2 * C, D), jnp.float32)
            y_scr[1, pl.ds(0, C), :] = kr * xr - ki * xi
            y_scr[1, pl.ds(C, C), :] = kr * xi + ki * xr

            def cmul_step(j, c):
                ma = ja - j
                mb = ma + 1
                for rc in range(C // RC):
                    r0 = rc * RC
                    xr = xf_scr[j, pl.ds(r0, RC), :]
                    xi = xf_scr[j, pl.ds(C + r0, RC), :]
                    kr = kf_scr[ma, pl.ds(r0, RC), :]
                    ki = kf_scr[ma, pl.ds(C + r0, RC), :]
                    y_scr[0, pl.ds(r0, RC), :] += kr * xr - ki * xi
                    y_scr[0, pl.ds(C + r0, RC), :] += kr * xi + ki * xr
                    kr = kf_scr[mb, pl.ds(r0, RC), :]
                    ki = kf_scr[mb, pl.ds(C + r0, RC), :]
                    y_scr[1, pl.ds(r0, RC), :] += kr * xr - ki * xi
                    y_scr[1, pl.ds(C + r0, RC), :] += kr * xi + ki * xr
                return c

            jax.lax.fori_loop(0, ja + 1, cmul_step, 0)

            finv = finv_ref[...]
            y = jnp.concatenate(
                [jnp.dot(finv, y_scr[0].astype(jnp.bfloat16),
                         preferred_element_type=jnp.float32),
                 jnp.dot(finv, y_scr[1].astype(jnp.bfloat16),
                         preferred_element_type=jnp.float32)], axis=0)
            y = y.astype(jnp.bfloat16).astype(jnp.float32)
            y = y + kv.astype(jnp.float32) * dv_ref[...]
            x = q_ref[...].astype(jnp.float32)
            h = x + _ln(x) * y
            row = pl.multiple_of(i * TM, TM)
            h_scr[pl.ds(row, TM), :] = h
            xb = _ln(h)
            xb_scr[pl.ds(row, TM), :] = xb
            u = _ln(xb).astype(jnp.bfloat16)
            @pl.when(i == 0)
            def _():
                wcopy(0).wait()

            hh = _gelu(jnp.dot(u, w1_scr[...], preferred_element_type=jnp.float32))
            hh_scr[pl.ds(pl.multiple_of(_HALO + i * TM, 8), TM), :] = hh

        @pl.when(i >= 1)
        def _phase_b():
            @pl.when(i == 1)
            def _():
                for n in range(1, 4):
                    wcopy(n).wait()
                for c0 in range(0, FF, 192):
                    w3_scr[:, c0:c0 + 192] = w3t_scr[c0:c0 + 192, :].astype(
                        jnp.float32).T.astype(w3_scr.dtype)

            b = i - 1
            row = pl.multiple_of(b * TM, TM)
            win = hh_scr[pl.ds(row, TM + 2 * _HALO), :]
            col = jax.lax.broadcasted_iota(jnp.int32, (TM, D), 1)
            hp1 = win[_HALO - 1:_HALO - 1 + TM]
            hm1 = win[_HALO + 1:_HALO + 1 + TM]
            hp2 = win[_HALO - 2:_HALO - 2 + TM]
            hm2 = win[_HALO + 2:_HALO + 2 + TM]
            g = jnp.where(col < c4, hp1,
                          jnp.where(col < 2 * c4, hm1,
                                    jnp.where(col < 3 * c4, hp2, hm2)))
            hs = jnp.dot(g.astype(jnp.bfloat16), w2_scr[...],
                         preferred_element_type=jnp.float32)
            h = h_scr[pl.ds(row, TM), :]
            xb = xb_scr[pl.ds(row, TM), :]
            x1 = xb + hs
            u = _ln(x1).astype(jnp.bfloat16)
            a = _gelu(jnp.dot(u, w3_scr[...], preferred_element_type=jnp.float32))
            h2 = jnp.dot(a.astype(jnp.bfloat16), w4_scr[...],
                         preferred_element_type=jnp.float32)
            out_ref[...] = (h + x1 + h2).astype(out_ref.dtype)

    return kernel


@jax.jit
def pallas_sequential_preLN__ssm_conv_h3__mixer_s_mlp__prompt_kernel(
    A_q: jax.Array,
    A_k: jax.Array,
    A_v: jax.Array,
    A_shift_k: jax.Array,
    A_ssm_k: jax.Array,
    A_ssm_D: jax.Array,
    B_x: jax.Array,
    B_w1: jax.Array,
    B_w2: jax.Array,
    B_w3: jax.Array,
    B_w4: jax.Array,
):
    B, S, D = A_q.shape
    assert B == 1
    FF = B_w3.shape[1]
    ks = A_shift_k.shape[1]
    assert ks == 4
    assert FF % 192 == 0
    C = 128
    TM = 2 * C
    RC = 8
    NT = S // TM
    NB = S // C

    q2 = A_q.reshape(S, D)
    k2 = A_k.reshape(S, D)
    v2 = A_v.reshape(S, D)
    kt = A_ssm_k
    sh = jnp.pad(A_shift_k.T.astype(jnp.float32), ((0, 8 - ks), (0, 0)))
    dv = A_ssm_D.reshape(1, D).astype(jnp.float32)
    fx_np, finv_np = _dft_mats(C)
    fx = jnp.asarray(fx_np, dtype=jnp.bfloat16)
    finv = jnp.asarray(finv_np, dtype=jnp.bfloat16)

    row_in = lambda i: (jnp.minimum(i, NT - 1), 0)
    col_in = lambda i: (0, jnp.minimum(i, NT - 1))
    row_out = lambda i: (jnp.maximum(i - 1, 0), 0)
    const = lambda i: (0, 0)

    kernel = _make_kernel(S, D, FF, C, TM, RC)
    out = pl.pallas_call(
        kernel,
        grid_spec=pltpu.PrefetchScalarGridSpec(
            num_scalar_prefetch=0,
            grid=(NT + 1,),
            in_specs=[
                pl.BlockSpec((TM, D), row_in),
                pl.BlockSpec((TM, D), row_in),
                pl.BlockSpec((TM, D), row_in),
                pl.BlockSpec((D, TM), col_in),
                pl.BlockSpec((8, D), const),
                pl.BlockSpec((1, D), const),
                pl.BlockSpec(memory_space=pl.ANY),
                pl.BlockSpec(memory_space=pl.ANY),
                pl.BlockSpec(memory_space=pl.ANY),
                pl.BlockSpec(memory_space=pl.ANY),
                pl.BlockSpec((2 * C, C), const),
                pl.BlockSpec((C, 2 * C), const),
            ],
            out_specs=pl.BlockSpec((TM, D), row_out),
            scratch_shapes=[
                pltpu.VMEM((NB, 2 * C, D), jnp.float32),
                pltpu.VMEM((NB, 2 * C, D), jnp.float32),
                pltpu.VMEM((2 * C, D), jnp.float32),
                pltpu.VMEM((8, D), jnp.float32),
                pltpu.VMEM((S, D), jnp.float32),
                pltpu.VMEM((S + 2 * _HALO, D), jnp.float32),
                pltpu.VMEM((2, 2 * C, D), jnp.float32),
                pltpu.VMEM((D, D), B_w1.dtype),
                pltpu.VMEM((D, D), B_w2.dtype),
                pltpu.VMEM((D, FF), B_w3.dtype),
                pltpu.VMEM((FF, D), B_w4.dtype),
                pltpu.SemaphoreType.DMA((4,)),
                pltpu.VMEM((FF, D), B_w3.dtype),
                pltpu.VMEM((S, D), jnp.float32),
            ],
        ),
        out_shape=jax.ShapeDtypeStruct((S, D), A_q.dtype),
        compiler_params=pltpu.CompilerParams(
            dimension_semantics=("arbitrary",),
            vmem_limit_bytes=120 * 1024 * 1024,
        ),
    )(q2, k2, v2, kt, sh, dv, B_w1, B_w2, B_w3.T, B_w4, fx, finv)
    return out.reshape(B, S, D)
```
